```python
import jax
import jax.numpy as jnp

def _softmax(x, axis=-1):
    return jax.nn.softmax(x, axis=axis)
def _gelu(x):
    return jax.nn.gelu(x, approximate=True)
def _silu(x):
    return jax.nn.silu(x)
def _sigmoid(x):
    return jax.nn.sigmoid(x)
def _layernorm(x, axis=-1, eps=1e-5):
    m = jnp.mean(x, axis=axis, keepdims=True)
    v = jnp.var(x, axis=axis, keepdims=True)
    return (x - m) / jnp.sqrt(v + eps)
def _scatter_add(tgt, idx, src, axis=0):
    return tgt.at[idx].add(src)
def _segment_sum(src, seg, n):
    return jax.ops.segment_sum(src, seg, n)
class _Rng:
    def __init__(self, key):
        self._k = key
    def _next(self):
        self._k, sub = jax.random.split(self._k)
        return sub
    def normal(self, shape):
        return jax.random.normal(self._next(), shape, dtype=jnp.bfloat16)
    def randint(self, lo, hi, shape):
        return jax.random.randint(self._next(), shape, lo, hi, dtype=jnp.int32)
    def uniform(self, shape, lo=0.0, hi=1.0):
        return jax.random.uniform(self._next(), shape, jnp.bfloat16, lo, hi)
    def permutation(self, n):
        return jax.random.permutation(self._next(), n)


kernel_name = 'recurrent_scan__sliding_block_cached__dense_activation_gelu__decode'

def setup_inputs():
    _rng = _Rng(jax.random.key(int.from_bytes(__import__("os").urandom(4), "little")))
    _w = (lambda a: (lambda t: t.astype(jnp.bfloat16) if jnp.issubdtype(t.dtype, jnp.floating) else t)(jnp.asarray(a)))
    def _A_setup():
        B, Sq, D = 2, 1, 576
        Hq, Hkv, Sk, Dh = 32, 16, 32768, 128
        assert Hq % Hkv == 0, (Hq, Hkv)
        return {
            "x": _w((lambda *s: _rng.normal(s) * 0.05)(B, Sq, D)),
            "k_cache": _w((lambda *s: _rng.normal(s) * 0.05)(B, Hkv, Sk, Dh)),
            "v_cache": _w((lambda *s: _rng.normal(s) * 0.05)(B, Hkv, Sk, Dh)),
            "wq": _w((lambda *s: _rng.normal(s) * 0.05)(D, Hq * Dh) * (D ** -0.5)),
            "wo": _w((lambda *s: _rng.normal(s) * 0.05)(Hq * Dh, D) * ((Hq * Dh) ** -0.5)),
        }
    _A_in = _A_setup()

    def _B_setup():
        B, S, D, F = 2, 1, 576, 4608
        return {
            "x": _w((lambda *s: _rng.normal(s) * 0.05)(B, S, D)),
            "w1": _w((lambda *s: _rng.normal(s) * 0.05)(D, F) * (D ** -0.5)),
            "b1": _w((lambda *s: _rng.normal(s) * 0.05)(F) * 0.01),
            "w2": _w((lambda *s: _rng.normal(s) * 0.05)(F, D) * (F ** -0.5)),
            "b2": _w((lambda *s: _rng.normal(s) * 0.05)(D) * 0.01),
        }
    _B_in = _B_setup()

    return {
        "A_x": _A_in["x"],
        "A_k_cache": _A_in["k_cache"],
        "A_v_cache": _A_in["v_cache"],
        "A_wq": _A_in["wq"],
        "A_wo": _A_in["wo"],
        "B_x": _B_in["x"],
        "B_w1": _B_in["w1"],
        "B_b1": _B_in["b1"],
        "B_w2": _B_in["w2"],
        "B_b2": _B_in["b2"],
    }

def reference(A_x, A_k_cache, A_v_cache, A_wq, A_wo, B_x, B_w1, B_b1, B_w2, B_b2):
    def _A_ref(x, k_cache, v_cache, wq, wo):
        B, Sq, D = x.shape
        Hq, Dh = 32, 128
        Hkv, Sk = k_cache.shape[1], k_cache.shape[2]
        W = min(4096, max(256, Sk // 4))
        rep = Hq // Hkv
        q = (lambda x, *d: x.transpose(*d))((x @ wq).reshape(B, Sq, Hq, Dh), 0, 2, 1, 3)
        k = jnp.repeat(k_cache[:, :, Sk - W:, :], rep, axis=1)
        v = jnp.repeat(v_cache[:, :, Sk - W:, :], rep, axis=1)
        scores = jnp.einsum("bhqd,bhkd->bhqk", q, k) * (Dh ** -0.5)
        p = _softmax(scores, axis=-1)
        o = jnp.einsum("bhqk,bhkd->bhqd", p, v)
        return (lambda x, *d: x.transpose(*d))(o, 0, 2, 1, 3).reshape(B, Sq, Hq * Dh) @ wo

    def _B_ref(x, w1, b1, w2, b2):
        h = jnp.einsum("bsd,df->bsf", x, w1) + b1
        h = _gelu(h)
        return jnp.einsum("bsf,fd->bsd", h, w2) + b2

    x = A_x
    xn = _layernorm(x, axis=-1)
    s = _A_ref(xn, A_k_cache, A_v_cache, A_wq, A_wo)
    g = _silu(_B_ref(xn, B_w1, B_b1, B_w2, B_b2))
    return x + s * g
```

```python
import functools
import jax
import jax.numpy as jnp
from jax import lax
import jax.experimental.pallas as pl
import jax.experimental.pallas.tpu as pltpu

NT = (((1,), (1,)), ((), ()))
F32, BF16 = jnp.float32, jnp.bfloat16


def make(NSLOT=4, vmem_mb=64):
    def kernel(x_hbm, k_hbm, v_hbm, wq_hbm, wo_hbm, w1_hbm, b1_hbm, w2_hbm, b2_hbm, o_ref,
               xb, b1b, b2b, kbuf, vbuf, wqb, wob, w1b, w2b, qs, ksem, vsem, wsem):
        B, Hkv, Sk, Dh = k_hbm.shape
        W = kbuf.shape[2]
        D = xb.shape[1]

        def kcp(h, slot):
            return pltpu.make_async_copy(k_hbm.at[:, h, pl.ds(Sk - W, W), :], kbuf.at[slot], ksem.at[slot])

        def vcp(h, slot):
            return pltpu.make_async_copy(v_hbm.at[:, h, pl.ds(Sk - W, W), :], vbuf.at[slot], vsem.at[slot])

        c_wq = pltpu.make_async_copy(wq_hbm, wqb, wsem.at[0])
        c_x = pltpu.make_async_copy(x_hbm, xb, wsem.at[1])
        c_b1 = pltpu.make_async_copy(b1_hbm, b1b, wsem.at[2])
        c_b2 = pltpu.make_async_copy(b2_hbm, b2b, wsem.at[3])
        c_w1 = pltpu.make_async_copy(w1_hbm, w1b, wsem.at[4])
        c_w2 = pltpu.make_async_copy(w2_hbm, w2b, wsem.at[5])
        c_wo = pltpu.make_async_copy(wo_hbm, wob, wsem.at[6])

        c_wq.start(); c_x.start(); c_b1.start(); c_b2.start()
        c_w1.start(); c_w2.start(); c_wo.start()
        for s in range(NSLOT):
            kcp(s, s).start(); vcp(s, s).start()

        c_x.wait()
        x = xb[...].astype(F32)
        m = jnp.mean(x, axis=-1, keepdims=True)
        xc = x - m
        var = jnp.mean(xc * xc, axis=-1, keepdims=True)
        xn = xc / jnp.sqrt(var + 1e-5)
        xn8 = jnp.concatenate([xn, xn, xn, xn], axis=0).astype(BF16)

        c_wq.wait()
        q = jnp.dot(xn8, wqb[...], preferred_element_type=F32)
        row = lax.broadcasted_iota(jnp.int32, (8, Dh), 0)
        for h in range(Hkv):
            qs[h] = jnp.where(row < 2, q[:, 2 * h * Dh:(2 * h + 1) * Dh], q[:, (2 * h + 1) * Dh:(2 * h + 2) * Dh])

        c_b1.wait(); c_w1.wait()
        hid = jnp.dot(xn8, w1b[...], preferred_element_type=F32) + b1b[...].astype(F32).reshape(1, -1)
        hid = jax.nn.gelu(hid, approximate=True).astype(BF16)
        c_b2.wait(); c_w2.wait()
        f = lax.dot_general(hid, w2b[...], NT, preferred_element_type=F32) + b2b[...].astype(F32).reshape(1, -1)
        g = f * jax.nn.sigmoid(f)
        c_wo.wait()

        scale = Dh ** -0.5

        def body(h, acc):
            slot = h % NSLOT
            qh = qs[h].astype(BF16)
            kcp(h, slot).wait()
            ps = []
            for b in range(B):
                s = lax.dot_general(qh, kbuf[slot, b], NT, preferred_element_type=F32) * scale
                mx = jnp.max(s, axis=-1, keepdims=True)
                p = jnp.exp(s - mx)
                l = jnp.sum(p, axis=-1, keepdims=True)
                ps.append((p.astype(BF16), l))

            @pl.when(h + NSLOT < Hkv)
            def _():
                kcp(h + NSLOT, slot).start()

            vcp(h, slot).wait()
            os_ = []
            for b in range(B):
                os_.append(jnp.dot(ps[b][0], vbuf[slot, b], preferred_element_type=F32) / ps[b][1])

            @pl.when(h + NSLOT < Hkv)
            def _():
                vcp(h + NSLOT, slot).start()

            o = jnp.where(row % 2 == 0, os_[0], os_[1])
            lhs = jnp.concatenate([jnp.where(row < 2, o, 0.0), jnp.where(row < 2, 0.0, o)], axis=1).astype(BF16)
            wsl = wob[:, pl.ds(pl.multiple_of(h * 2 * Dh, 2 * Dh), 2 * Dh)]
            return acc + lax.dot_general(lhs, wsl, NT, preferred_element_type=F32)

        acc = lax.fori_loop(0, Hkv, body, jnp.zeros((8, D), F32))
        s = acc[0:2] + acc[2:4]
        o_ref[...] = (x + s * g[0:2]).astype(o_ref.dtype)

    @jax.jit
    def fn(A_x, A_k_cache, A_v_cache, A_wq, A_wo, B_x, B_w1, B_b1, B_w2, B_b2):
        B, Sq, D = A_x.shape
        _, Hkv, Sk, Dh = A_k_cache.shape
        W = min(4096, max(256, Sk // 4))
        F = B_w1.shape[1]
        HD = A_wq.shape[1]
        out = pl.pallas_call(
            kernel,
            out_shape=jax.ShapeDtypeStruct((B, D), A_x.dtype),
            in_specs=[pl.BlockSpec(memory_space=pl.ANY)] * 9,
            out_specs=pl.BlockSpec(memory_space=pltpu.VMEM),
            scratch_shapes=[
                pltpu.VMEM((B, D), BF16), pltpu.VMEM((F,), BF16), pltpu.VMEM((D,), BF16),
                pltpu.VMEM((NSLOT, B, W, Dh), BF16), pltpu.VMEM((NSLOT, B, W, Dh), BF16),
                pltpu.VMEM((D, HD), BF16), pltpu.VMEM((D, HD), BF16),
                pltpu.VMEM((D, F), BF16), pltpu.VMEM((D, F), BF16),
                pltpu.VMEM((Hkv, 8, Dh), F32),
                pltpu.SemaphoreType.DMA((NSLOT,)), pltpu.SemaphoreType.DMA((NSLOT,)),
                pltpu.SemaphoreType.DMA((7,)),
            ],
            compiler_params=pltpu.CompilerParams(vmem_limit_bytes=vmem_mb * 1024 * 1024),
        )(A_x.reshape(B, D), A_k_cache, A_v_cache, A_wq, A_wo.T, B_w1, B_b1, B_w2.T, B_b2)
        return out.reshape(B, Sq, D)
    return fn


pallas_recurrent_scan__sliding_block_cached__dense_activation_gelu__decode_kernel = make()
```

```python
import functools
import jax
import jax.numpy as jnp
from jax import lax
import jax.experimental.pallas as pl
import jax.experimental.pallas.tpu as pltpu

NT = (((1,), (1,)), ((), ()))
F32, BF16 = jnp.float32, jnp.bfloat16


def make(NSLOT=3, R=128, ZS=(256, 128, 128, 64), vmem_mb=64, nochk=False, HG=2):
    def kernel(x_hbm, k_hbm, v_hbm, wq_hbm, wo_hbm, w1_hbm, b1_hbm, w2_hbm, b2_hbm, o_ref,
               xb, b1b, b2b, kbuf, vbuf, wqb, wob, w1b, w2b, qs, os_, ksem, vsem, wsem):
        B, Hkv, Sk, Dh = k_hbm.shape
        W = kbuf.shape[3]
        D = xb.shape[1]
        NG = Hkv // HG

        def start_kv(g, slot, p0=0, n=W // R):
            def body(p, c):
                r = pl.multiple_of(p * R, R)
                for hh in range(HG):
                    for b in range(B):
                        for q, (src, dst, sem) in enumerate(((k_hbm, kbuf, ksem), (v_hbm, vbuf, vsem))):
                            pltpu.make_async_copy(src.at[b, g * HG + hh, pl.ds(Sk - W + r, R), :],
                                                  dst.at[slot, hh, b, pl.ds(r, R), :], sem.at[slot]).start(priority=q)
                return c
            lax.fori_loop(p0, p0 + n, body, 0)

        def start_w(pairs, row0, nrows, i0=0, n=None, ns=4):
            rs = nrows // ns
            def body(i, c):
                for cc in range(3):
                    for s in range(ns):
                        for q, (src, dst, sem) in enumerate(pairs):
                            N = src.shape[1]
                            nc = 2 if N % 2048 == 0 else 3
                            if cc >= nc:
                                continue
                            cw = N // nc
                            r = pl.multiple_of(row0 + s * rs + i * 8, 8)
                            pltpu.make_async_copy(src.at[pl.ds(r, 8), pl.ds(cc * cw, cw)],
                                                  dst.at[pl.ds(r, 8), pl.ds(cc * cw, cw)], sem).start(priority=q)
                return c
            lax.fori_loop(i0, i0 + (n or rs // 8), body, 0)

        def wait_all(ref, sem):
            pltpu.make_async_copy(ref, ref, sem).wait()

        c_x = pltpu.make_async_copy(x_hbm, xb, wsem.at[0])
        c_b1 = pltpu.make_async_copy(b1_hbm, b1b, wsem.at[1])
        c_b2 = pltpu.make_async_copy(b2_hbm, b2b, wsem.at[2])
        start_w(((wq_hbm, wqb, wsem.at[3]), (w1_hbm, w1b, wsem.at[4])), 0, D)
        c_x.start(); c_b1.start(); c_b2.start()
        start_kv(0, 0)

        c_x.wait()
        x = xb[...].astype(F32)
        m = jnp.mean(x, axis=-1, keepdims=True)
        xc = x - m
        var = jnp.mean(xc * xc, axis=-1, keepdims=True)
        xn = xc / jnp.sqrt(var + 1e-5)
        xn8 = jnp.concatenate([xn, xn, xn, xn], axis=0).astype(BF16)

        wait_all(wqb, wsem.at[3])
        q = jnp.dot(xn8, wqb[...], preferred_element_type=F32)
        row = lax.broadcasted_iota(jnp.int32, (8, Dh), 0)
        for h in range(Hkv):
            qs[h] = jnp.where(row < 2, q[:, 2 * h * Dh:(2 * h + 1) * Dh], q[:, (2 * h + 1) * Dh:(2 * h + 2) * Dh])

        start_kv(1, 1, 0, W // R // 2)
        c_b1.wait(); wait_all(w1b, wsem.at[4])
        hid = jnp.dot(xn8, w1b[...], preferred_element_type=F32) + b1b[...].astype(F32).reshape(1, -1)
        hid = jax.nn.gelu(hid, approximate=True).astype(BF16)
        c_b2.wait()
        start_kv(1, 1, W // R // 2, W // R // 2)

        scale = Dh ** -0.5
        NP = HG * B
        zp = lambda i: ((w2_hbm, w2b, wsem.at[5 + 2 * i]), (wo_hbm, wob, wsem.at[6 + 2 * i]))

        def body(g, carry):
            slot = g % NSLOT
            wait_all(kbuf.at[slot], ksem.at[slot])
            wait_all(vbuf.at[slot], vsem.at[slot])
            for hh in range(HG):
                h = g * HG + hh
                qh = qs[h].astype(BF16)
                outs = []
                for b in range(B):
                    s = lax.dot_general(qh, kbuf[slot, hh, b], NT, preferred_element_type=F32) * scale
                    mx = jnp.max(s, axis=-1, keepdims=True)
                    p = jnp.exp(s - mx)
                    l = jnp.sum(p, axis=-1, keepdims=True)
                    outs.append(jnp.dot(p.astype(BF16), vbuf[slot, hh, b], preferred_element_type=F32) / l)
                    j = hh * B + b

                    @pl.when(g + 2 < NG)
                    def _():
                        start_kv(g + 2, (g + 2) % NSLOT, j * (W // R // NP), W // R // NP)

                    @pl.when(g + 2 >= NG)
                    def _():
                        nz = ZS[0] // 4 // 8 // (2 * NP)
                        start_w(zp(0), 0, ZS[0], ((g + 2 - NG) * NP + j) * nz, nz)
                o = jnp.where(row % 2 == 0, outs[0], outs[1])
                os_[:, pl.ds(pl.multiple_of(h * 2 * Dh, 2 * Dh), 2 * Dh)] = jnp.concatenate([o, pltpu.roll(o, 6, 0)], axis=1)

            return carry

        lax.fori_loop(0, NG, body, 0)
        ob = os_[...].astype(BF16)
        b2 = b2b[...].astype(F32).reshape(1, -1)
        for i, n in enumerate(ZS):
            r0, s2, so = sum(ZS[:i]), 5 + 2 * i, 6 + 2 * i
            if i + 1 < len(ZS):
                start_w(zp(i + 1), r0 + n, ZS[i + 1])
            wait_all(w2b.at[pl.ds(r0, n)], wsem.at[s2])
            f = lax.dot_general(hid, w2b[r0:r0 + n, :], NT, preferred_element_type=F32) + b2[:, r0:r0 + n]
            gte = f * jax.nn.sigmoid(f)
            wait_all(wob.at[pl.ds(r0, n)], wsem.at[so])
            s = lax.dot_general(ob, wob[r0:r0 + n, :], NT, preferred_element_type=F32)
            o_ref[:, r0:r0 + n] = (x[:, r0:r0 + n] + (s * gte)[0:2]).astype(o_ref.dtype)

    @jax.jit
    def fn(A_x, A_k_cache, A_v_cache, A_wq, A_wo, B_x, B_w1, B_b1, B_w2, B_b2):
        B, Sq, D = A_x.shape
        _, Hkv, Sk, Dh = A_k_cache.shape
        W = min(4096, max(256, Sk // 4))
        F = B_w1.shape[1]
        HD = A_wq.shape[1]
        out = pl.pallas_call(
            kernel,
            out_shape=jax.ShapeDtypeStruct((B, D), A_x.dtype),
            in_specs=[pl.BlockSpec(memory_space=pl.ANY)] * 9,
            out_specs=pl.BlockSpec(memory_space=pltpu.VMEM),
            scratch_shapes=[
                pltpu.VMEM((B, D), BF16), pltpu.VMEM((F,), BF16), pltpu.VMEM((D,), BF16),
                pltpu.VMEM((NSLOT, HG, B, W, Dh), BF16), pltpu.VMEM((NSLOT, HG, B, W, Dh), BF16),
                pltpu.VMEM((D, HD), BF16), pltpu.VMEM((D, HD), BF16),
                pltpu.VMEM((D, F), BF16), pltpu.VMEM((D, F), BF16),
                pltpu.VMEM((Hkv, 8, Dh), F32), pltpu.VMEM((8, HD), F32),
                pltpu.SemaphoreType.DMA((NSLOT,)), pltpu.SemaphoreType.DMA((NSLOT,)),
                pltpu.SemaphoreType.DMA((5 + 2 * len(ZS),)),
            ],
            compiler_params=pltpu.CompilerParams(vmem_limit_bytes=vmem_mb * 1024 * 1024, disable_bounds_checks=nochk),
        )(A_x.reshape(B, D), A_k_cache, A_v_cache, A_wq, A_wo.T, B_w1, B_b1, B_w2.T, B_b2)
        return out.reshape(B, Sq, D)
    return fn


pallas_recurrent_scan__sliding_block_cached__dense_activation_gelu__decode_kernel = make(nochk=True)
```

```python
import functools
import jax
import jax.numpy as jnp
from jax import lax
import jax.experimental.pallas as pl
import jax.experimental.pallas.tpu as pltpu

NT = (((1,), (1,)), ((), ()))
F32, BF16 = jnp.float32, jnp.bfloat16


def make(NSLOT=3, R=128, ZS=(256, 128, 128, 64), vmem_mb=64, nochk=False, HG=4, sk=0, sv=0):
    def kernel(x_hbm, k_hbm, v_hbm, wq_hbm, wo_hbm, w1_hbm, b1_hbm, w2_hbm, b2_hbm, o_ref,
               xb, b1b, b2b, kbuf, vbuf, wqb, wob, w1b, w2b, qs, os_, ksem, vsem, wsem):
        B, Hkv, Sk, Dh = k_hbm.shape
        W = kbuf.shape[2]
        D = xb.shape[1]
        NGB = Hkv // HG
        NG = B * NGB
        shifts = (sk, sv)

        def kv_rows(g, slot, r0, n):
            for hh in range(HG):
                for q, (src, dst, sem) in enumerate(((k_hbm, kbuf, ksem), (v_hbm, vbuf, vsem))):
                    r, nn = r0[q], n[q]
                    if nn:
                        pltpu.make_async_copy(src.at[g // NGB, (g % NGB) * HG + hh, pl.ds(Sk - W + r, nn), :],
                                              dst.at[slot, hh, pl.ds(r, nn), :], sem.at[slot]).start(priority=q)

        def start_kv(g, slot, p0=0, n=W // R):
            last = p0 + n == W // R
            def body(p, c):
                kv_rows(g, slot, [pl.multiple_of(p * R + s, 2) for s in shifts], (R, R))
                return c
            lax.fori_loop(p0, p0 + n - last, body, 0)
            if last:
                kv_rows(g, slot, [W - R + s for s in shifts], [R - s for s in shifts])
                kv_rows(g, slot, (0, 0), shifts)

        def start_w(pairs, row0, nrows, i0=0, n=None, ns=4):
            rs = nrows // ns
            def body(i, c):
                for cc in range(3):
                    for s in range(ns):
                        for q, (src, dst, sem) in enumerate(pairs):
                            N = src.shape[1]
                            nc = 2 if N % 2048 == 0 else 3
                            if cc >= nc:
                                continue
                            cw = N // nc
                            r = pl.multiple_of(row0 + s * rs + i * 8, 8)
                            pltpu.make_async_copy(src.at[pl.ds(r, 8), pl.ds(cc * cw, cw)],
                                                  dst.at[pl.ds(r, 8), pl.ds(cc * cw, cw)], sem).start(priority=q)
                return c
            lax.fori_loop(i0, i0 + (n or rs // 8), body, 0)

        def wait_all(ref, sem):
            pltpu.make_async_copy(ref, ref, sem).wait()

        c_x = pltpu.make_async_copy(x_hbm, xb, wsem.at[0])
        c_b1 = pltpu.make_async_copy(b1_hbm, b1b, wsem.at[1])
        c_b2 = pltpu.make_async_copy(b2_hbm, b2b, wsem.at[2])
        start_w(((wq_hbm, wqb, wsem.at[3]), (w1_hbm, w1b, wsem.at[4])), 0, D)
        c_x.start(); c_b1.start(); c_b2.start()
        start_kv(0, 0)

        os_[...] = jnp.zeros(os_.shape, F32)
        c_x.wait()
        x = xb[...].astype(F32)
        m = jnp.mean(x, axis=-1, keepdims=True)
        xc = x - m
        var = jnp.mean(xc * xc, axis=-1, keepdims=True)
        xn = xc / jnp.sqrt(var + 1e-5)
        xn8 = jnp.concatenate([xn, xn, xn, xn], axis=0).astype(BF16)

        wait_all(wqb, wsem.at[3])
        q = jnp.dot(xn8, wqb[...], preferred_element_type=F32)
        row = lax.broadcasted_iota(jnp.int32, (8, Dh), 0)
        for h in range(Hkv):
            qs[h] = jnp.where(row < 2, q[:, 2 * h * Dh:(2 * h + 1) * Dh], q[:, (2 * h + 1) * Dh:(2 * h + 2) * Dh])

        start_kv(1, 1, 0, W // R // 2)
        c_b1.wait(); wait_all(w1b, wsem.at[4])
        hid = (jnp.dot(xn8, w1b[...], preferred_element_type=F32)) + b1b[...].astype(F32).reshape(1, -1)
        hid = jax.nn.gelu(hid, approximate=True).astype(BF16)
        c_b2.wait()
        start_kv(1, 1, W // R // 2, W // R // 2)

        scale = Dh ** -0.5
        NP = HG
        zp = lambda i: ((w2_hbm, w2b, wsem.at[5 + 2 * i]), (wo_hbm, wob, wsem.at[6 + 2 * i]))

        def body(g, carry):
            slot = g % NSLOT
            wait_all(kbuf.at[slot], ksem.at[slot])
            wait_all(vbuf.at[slot], vsem.at[slot])
            b = g // NGB
            for j in range(HG):
                if True:
                    h = (g % NGB) * HG + j
                    qh = qs[h].astype(BF16)
                    s = lax.dot_general(qh, kbuf[slot, j], NT, preferred_element_type=F32) * scale
                    mx = jnp.max(s, axis=-1, keepdims=True)
                    p = jnp.exp(s - mx)
                    l = jnp.sum(p, axis=-1, keepdims=True)
                    o = jnp.dot(p.astype(BF16), vbuf[slot, j], preferred_element_type=F32) / l
                    cols = pl.ds(pl.multiple_of(h * 2 * Dh, 2 * Dh), 2 * Dh)
                    o2 = jnp.concatenate([o, pltpu.roll(o, 6, 0)], axis=1)
                    os_[:, cols] = jnp.where(lax.broadcasted_iota(jnp.int32, o2.shape, 0) == b, o2, os_[:, cols])

                    @pl.when(g + 2 < NG)
                    def _():
                        start_kv(g + 2, (g + 2) % NSLOT, j * (W // R // NP), W // R // NP)

                    @pl.when(g + 2 >= NG)
                    def _():
                        nz = ZS[0] // 4 // 8 // (2 * NP)
                        start_w(zp(0), 0, ZS[0], ((g + 2 - NG) * NP + j) * nz, nz)
            return carry

        lax.fori_loop(0, NG, body, 0)
        ob = os_[...].astype(BF16)
        b2 = b2b[...].astype(F32).reshape(1, -1)
        for i, n in enumerate(ZS):
            r0, s2, so = sum(ZS[:i]), 5 + 2 * i, 6 + 2 * i
            if i + 1 < len(ZS):
                start_w(zp(i + 1), r0 + n, ZS[i + 1])
            wait_all(w2b.at[pl.ds(r0, n)], wsem.at[s2])
            f = (lax.dot_general(hid, w2b[r0:r0 + n, :], NT, preferred_element_type=F32)) + b2[:, r0:r0 + n]
            gte = f * jax.nn.sigmoid(f)
            wait_all(wob.at[pl.ds(r0, n)], wsem.at[so])
            s = lax.dot_general(ob, wob[r0:r0 + n, :], NT, preferred_element_type=F32)
            o_ref[:, r0:r0 + n] = (x[:, r0:r0 + n] + (s * gte)[0:2]).astype(o_ref.dtype)

    @jax.jit
    def fn(A_x, A_k_cache, A_v_cache, A_wq, A_wo, B_x, B_w1, B_b1, B_w2, B_b2):
        B, Sq, D = A_x.shape
        _, Hkv, Sk, Dh = A_k_cache.shape
        W = min(4096, max(256, Sk // 4))
        F = B_w1.shape[1]
        HD = A_wq.shape[1]
        out = pl.pallas_call(
            kernel,
            out_shape=jax.ShapeDtypeStruct((B, D), A_x.dtype),
            in_specs=[pl.BlockSpec(memory_space=pl.ANY)] * 9,
            out_specs=pl.BlockSpec(memory_space=pltpu.VMEM),
            scratch_shapes=[
                pltpu.VMEM((B, D), BF16), pltpu.VMEM((F,), BF16), pltpu.VMEM((D,), BF16),
                pltpu.VMEM((NSLOT, HG, W, Dh), BF16), pltpu.VMEM((NSLOT, HG, W, Dh), BF16),
                pltpu.VMEM((D, HD), BF16), pltpu.VMEM((D, HD), BF16),
                pltpu.VMEM((D, F), BF16), pltpu.VMEM((D, F), BF16),
                pltpu.VMEM((Hkv, 8, Dh), F32), pltpu.VMEM((8, HD), F32),
                pltpu.SemaphoreType.DMA((NSLOT,)), pltpu.SemaphoreType.DMA((NSLOT,)),
                pltpu.SemaphoreType.DMA((5 + 2 * len(ZS),)),
            ],
            compiler_params=pltpu.CompilerParams(vmem_limit_bytes=vmem_mb * 1024 * 1024, disable_bounds_checks=nochk),
        )(A_x.reshape(B, D), A_k_cache, A_v_cache, A_wq, A_wo.T, B_w1, B_b1, B_w2.T, B_b2)
        return out.reshape(B, Sq, D)
    return fn


pallas_recurrent_scan__sliding_block_cached__dense_activation_gelu__decode_kernel = make(nochk=True, sk=0, sv=64)
```

```python
import functools
import jax
import jax.numpy as jnp
from jax import lax
import jax.experimental.pallas as pl
import jax.experimental.pallas.tpu as pltpu

NT = (((1,), (1,)), ((), ()))
F32, BF16 = jnp.float32, jnp.bfloat16


def make(NSLOT=3, R=128, Z0=256, Z1=512, CS=3072, vmem_mb=64, nochk=False, HG=4, sk=0, sv=0, nosem=False):
    def kernel(x_hbm, k_hbm, v_hbm, wq_hbm, wo_hbm, w1_hbm, b1_hbm, w2_hbm, b2_hbm, o_ref,
               xb, b1b, b2b, kbuf, vbuf, wqb, wob, w1b, w2b, qs, os_, ksem, vsem, wsem):
        B, Hkv, Sk, Dh = k_hbm.shape
        W = kbuf.shape[2]
        D = xb.shape[1]
        NGB = Hkv // HG
        NG = B * NGB
        shifts = (sk, sv)

        def kv_rows(g, slot, r0, n):
            for hh in range(HG):
                for q, (src, dst, sem) in enumerate(((k_hbm, kbuf, ksem), (v_hbm, vbuf, vsem))):
                    r, nn = r0[q], n[q]
                    if nn:
                        pltpu.make_async_copy(src.at[g // NGB, (g % NGB) * HG + hh, pl.ds(Sk - W + r, nn), :],
                                              dst.at[slot, hh, pl.ds(r, nn), :], sem.at[slot]).start(priority=q)

        def start_kv(g, slot, p0=0, n=W // R):
            last = p0 + n == W // R
            def body(p, c):
                kv_rows(g, slot, [pl.multiple_of(p * R + s, 2) for s in shifts], (R, R))
                return c
            lax.fori_loop(p0, p0 + n - last, body, 0)
            if last:
                kv_rows(g, slot, [W - R + s for s in shifts], [R - s for s in shifts])
                kv_rows(g, slot, (0, 0), shifts)

        def start_w(pairs, nrows, i0=0, n=None, ns=4):
            rs = nrows // ns
            def body(i, c):
                for cc in range(3):
                    for s in range(ns):
                        for q, (src, dst, sem, row0, c0, c1) in enumerate(pairs):
                            nc = -(-(c1 - c0) // 2048)
                            if cc >= nc:
                                continue
                            cw = (c1 - c0) // nc
                            r = pl.multiple_of(row0 + s * rs + i * 8, 8)
                            pltpu.make_async_copy(src.at[pl.ds(r, 8), pl.ds(c0 + cc * cw, cw)],
                                                  dst.at[pl.ds(r, 8), pl.ds(c0 + cc * cw, cw)], sem).start(priority=q)
                return c
            n = n or rs // 8
            if n == 1:
                body(i0, 0)
            else:
                lax.fori_loop(i0, i0 + n, body, 0)

        def wait_all(ref, sem):
            pltpu.make_async_copy(ref, ref, sem).wait()

        c_x = pltpu.make_async_copy(x_hbm, xb, wsem.at[0])
        c_b1 = pltpu.make_async_copy(b1_hbm, b1b, wsem.at[1])
        c_b2 = pltpu.make_async_copy(b2_hbm, b2b, wsem.at[2])
        F, HD = w1_hbm.shape[1], wq_hbm.shape[1]
        start_w(((wq_hbm, wqb, wsem.at[3], 0, 0, HD), (w1_hbm, w1b, wsem.at[4], 0, 0, F)), D)
        c_x.start(); c_b1.start(); c_b2.start()
        start_kv(0, 0)

        os_[...] = jnp.zeros(os_.shape, F32)
        c_x.wait()
        x = xb[...].astype(F32)
        m = jnp.mean(x, axis=-1, keepdims=True)
        xc = x - m
        var = jnp.mean(xc * xc, axis=-1, keepdims=True)
        xn = xc / jnp.sqrt(var + 1e-5)
        xn8 = jnp.concatenate([xn, xn, xn, xn], axis=0).astype(BF16)

        wait_all(wqb, wsem.at[3])
        q = jnp.dot(xn8, wqb[...], preferred_element_type=F32)
        row = lax.broadcasted_iota(jnp.int32, (8, Dh), 0)
        for h in range(Hkv):
            qs[h] = jnp.where(row < 2, q[:, 2 * h * Dh:(2 * h + 1) * Dh], q[:, (2 * h + 1) * Dh:(2 * h + 2) * Dh])

        start_kv(1, 1, 0, W // R // 2)
        c_b1.wait(); wait_all(w1b, wsem.at[4])
        hid = (jnp.dot(xn8, w1b[...], preferred_element_type=F32)) + b1b[...].astype(F32).reshape(1, -1)
        hid = jax.nn.gelu(hid, approximate=True).astype(BF16)
        c_b2.wait()
        start_kv(1, 1, W // R // 2, W // R // 2)

        scale = Dh ** -0.5
        NP = HG

        def body(g, carry):
            slot = g % NSLOT
            wait_all(kbuf.at[slot], ksem.at[slot])
            wait_all(vbuf.at[slot], vsem.at[slot])
            b = g // NGB
            for j in range(HG):
                if True:
                    h = (g % NGB) * HG + j
                    qh = qs[h].astype(BF16)
                    s = lax.dot_general(qh, kbuf[slot, j], NT, preferred_element_type=F32) * scale
                    mx = jnp.max(s, axis=-1, keepdims=True)
                    p = jnp.exp(s - mx)
                    l = jnp.sum(p, axis=-1, keepdims=True)
                    o = jnp.dot(p.astype(BF16), vbuf[slot, j], preferred_element_type=F32) / l
                    cols = pl.ds(pl.multiple_of(h * 2 * Dh, 2 * Dh), 2 * Dh)
                    o2 = jnp.concatenate([o, pltpu.roll(o, 6, 0)], axis=1)
                    os_[:, cols] = jnp.where(lax.broadcasted_iota(jnp.int32, o2.shape, 0) == b, o2, os_[:, cols])

                    @pl.when(g + 2 < NG)
                    def _():
                        start_kv(g + 2, (g + 2) % NSLOT, j * (W // R // NP), W // R // NP)

                    @pl.when(g + 2 >= NG)
                    def _():
                        nz = Z0 // 4 // 8 // (2 * NP)
                        start_w(((w2_hbm, w2b, wsem.at[5], 0, 0, F), (wo_hbm, wob, wsem.at[6], 0, 0, HD)), Z0, ((g + 2 - NG) * NP + j) * nz, nz)
            return carry

        lax.fori_loop(0, NG, body, 0)
        ob = os_[...].astype(BF16)
        b2 = b2b[...].astype(F32).reshape(1, -1)
        def gate(r0, r1):
            f = lax.dot_general(hid, w2b[r0:r1, :], NT, preferred_element_type=F32) + b2[:, r0:r1]
            return f * jax.nn.sigmoid(f)

        def proj(r0, r1, c0=0, c1=HD):
            return lax.dot_general(ob[:, c0:c1], wob[r0:r1, c0:c1], NT, preferred_element_type=F32)

        def emit(r0, r1, s, g):
            o_ref[:, r0:r1] = (x[:, r0:r1] + (s * g)[0:2]).astype(o_ref.dtype)

        def split(src, dst, sem, r0, r1, c0, c1, i0=0, n=None):
            h = (r1 - r0) // 2
            start_w(((src, dst, sem, r0, c0, c1), (src, dst, sem, r0 + h, c0, c1)), h, i0, n)

        split(w2_hbm, w2b, wsem.at[7], Z0, D, 0, F, 0, 3)
        wait_all(w2b.at[pl.ds(0, Z0)], wsem.at[5])
        g0 = gate(0, Z0)
        split(w2_hbm, w2b, wsem.at[7], Z0, D, 0, F, 3, 2)
        wait_all(wob.at[pl.ds(0, Z0)], wsem.at[6])
        emit(0, Z0, proj(0, Z0), g0)
        split(wo_hbm, wob, wsem.at[8], 256, 384, 0, HD)
        split(wo_hbm, wob, wsem.at[9], 384, 512, 0, HD)
        wait_all(w2b.at[pl.ds(Z0, D - Z0)], wsem.at[7])
        g1 = gate(Z0, D)
        if CS:
            split(wo_hbm, wob, wsem.at[10], 512, D, 0, CS)
        split(wo_hbm, wob, wsem.at[11], 512, D, CS, HD)
        wait_all(wob.at[pl.ds(256, 128)], wsem.at[8])
        emit(256, 384, proj(256, 384), g1[:, 0:128])
        wait_all(wob.at[pl.ds(384, 128)], wsem.at[9])
        emit(384, 512, proj(384, 512), g1[:, 128:256])
        s = 0.0
        if CS:
            wait_all(wob.at[pl.ds(512, 64), pl.ds(0, CS)], wsem.at[10])
            qs[0, :, 0:64] = proj(512, D, 0, CS)
        wait_all(wob.at[pl.ds(512, 64), pl.ds(CS, HD - CS)], wsem.at[11])
        if CS:
            s = qs[0, :, 0:64]
        emit(512, D, s + proj(512, D, CS, HD), g1[:, 256:])

    @jax.jit
    def fn(A_x, A_k_cache, A_v_cache, A_wq, A_wo, B_x, B_w1, B_b1, B_w2, B_b2):
        B, Sq, D = A_x.shape
        _, Hkv, Sk, Dh = A_k_cache.shape
        W = min(4096, max(256, Sk // 4))
        F = B_w1.shape[1]
        HD = A_wq.shape[1]
        out = pl.pallas_call(
            kernel,
            out_shape=jax.ShapeDtypeStruct((B, D), A_x.dtype),
            in_specs=[pl.BlockSpec(memory_space=pl.ANY)] * 9,
            out_specs=pl.BlockSpec(memory_space=pltpu.VMEM),
            scratch_shapes=[
                pltpu.VMEM((B, D), BF16), pltpu.VMEM((F,), BF16), pltpu.VMEM((D,), BF16),
                pltpu.VMEM((NSLOT, HG, W, Dh), BF16), pltpu.VMEM((NSLOT, HG, W, Dh), BF16),
                pltpu.VMEM((D, HD), BF16), pltpu.VMEM((D, HD), BF16),
                pltpu.VMEM((D, F), BF16), pltpu.VMEM((D, F), BF16),
                pltpu.VMEM((Hkv, 8, Dh), F32), pltpu.VMEM((8, HD), F32),
                pltpu.SemaphoreType.DMA((NSLOT,)), pltpu.SemaphoreType.DMA((NSLOT,)),
                pltpu.SemaphoreType.DMA((12,)),
            ],
            compiler_params=pltpu.CompilerParams(vmem_limit_bytes=vmem_mb * 1024 * 1024, disable_bounds_checks=nochk, disable_semaphore_checks=nosem),
        )(A_x.reshape(B, D), A_k_cache, A_v_cache, A_wq, A_wo.T, B_w1, B_b1, B_w2.T, B_b2)
        return out.reshape(B, Sq, D)
    return fn


pallas_recurrent_scan__sliding_block_cached__dense_activation_gelu__decode_kernel = make(nochk=True, CS=0, nosem=True, sk=0, sv=64)
```

```python
import jax
import jax.numpy as jnp
from jax import lax
import jax.experimental.pallas as pl
import jax.experimental.pallas.tpu as pltpu

F32, BF16 = jnp.float32, jnp.bfloat16
NT = (((1,), (1,)), ((), ()))

NSLOT = 3
HG = 4
R = 128
SHIFT = (0, 64)
Z0 = 256


def _kernel(x_hbm, k_hbm, v_hbm, wq_hbm, wo_hbm, w1_hbm, b1_hbm, w2_hbm, b2_hbm, o_ref,
            xb, b1b, b2b, kbuf, vbuf, wqb, wob, w1b, w2b, qs, os_, ksem, vsem, wsem):
    B, Hkv, Sk, Dh = k_hbm.shape
    W = kbuf.shape[2]
    D, HD = wqb.shape
    NGB = Hkv // HG
    NG = B * NGB
    NC = W // R

    def kv_rows(g, slot, r0, n):
        for hh in range(HG):
            for q, (src, dst, sem) in enumerate(((k_hbm, kbuf, ksem), (v_hbm, vbuf, vsem))):
                if n[q]:
                    pltpu.make_async_copy(
                        src.at[g // NGB, (g % NGB) * HG + hh, pl.ds(Sk - W + r0[q], n[q]), :],
                        dst.at[slot, hh, pl.ds(r0[q], n[q]), :],
                        sem.at[slot]).start(priority=q)

    def start_kv(g, slot, p0=0, n=NC):
        last = p0 + n == NC

        def body(p, c):
            kv_rows(g, slot, [pl.multiple_of(p * R + s, 16) for s in SHIFT], (R, R))
            return c
        lax.fori_loop(p0, p0 + n - last, body, 0)
        if last:
            kv_rows(g, slot, [W - R + s for s in SHIFT], [R - s for s in SHIFT])
            kv_rows(g, slot, (0, 0), SHIFT)

    def start_w(jobs, nrows, i0=0, n=None, ns=4):
        rs = nrows // ns

        def body(i, c):
            for cc in range(3):
                for s in range(ns):
                    for q, (src, dst, sem, row0) in enumerate(jobs):
                        nc = pl.cdiv(src.shape[1], 2048)
                        if cc < nc:
                            cw = src.shape[1] // nc
                            r = pl.multiple_of(row0 + s * rs + i * 8, 8)
                            idx = (pl.ds(r, 8), pl.ds(cc * cw, cw))
                            pltpu.make_async_copy(src.at[idx], dst.at[idx], sem).start(priority=q)
            return c
        n = n or rs // 8
        if n == 1:
            body(i0, 0)
        else:
            lax.fori_loop(i0, i0 + n, body, 0)

    def start_rows(src, dst, sem, r0, r1, i0=0, n=None):
        h = (r1 - r0) // 2
        start_w(((src, dst, sem, r0), (src, dst, sem, r0 + h)), h, i0, n)

    def wait_all(ref, sem):
        pltpu.make_async_copy(ref, ref, sem).wait()

    c_x = pltpu.make_async_copy(x_hbm, xb, wsem.at[0])
    c_b1 = pltpu.make_async_copy(b1_hbm, b1b, wsem.at[1])
    c_b2 = pltpu.make_async_copy(b2_hbm, b2b, wsem.at[2])
    start_w(((wq_hbm, wqb, wsem.at[3], 0), (w1_hbm, w1b, wsem.at[4], 0)), D)
    c_x.start()
    c_b1.start()
    c_b2.start()
    start_kv(0, 0)

    os_[...] = jnp.zeros(os_.shape, F32)
    c_x.wait()
    x = xb[...].astype(F32)
    xc = x - jnp.mean(x, axis=-1, keepdims=True)
    xn = xc / jnp.sqrt(jnp.mean(xc * xc, axis=-1, keepdims=True) + 1e-5)
    xn8 = jnp.concatenate([xn] * 4, axis=0).astype(BF16)

    wait_all(wqb, wsem.at[3])
    q = jnp.dot(xn8, wqb[...], preferred_element_type=F32)
    row = lax.broadcasted_iota(jnp.int32, (8, Dh), 0)
    for h in range(Hkv):
        qs[h] = jnp.where(row < 2, q[:, 2 * h * Dh:(2 * h + 1) * Dh],
                          q[:, (2 * h + 1) * Dh:(2 * h + 2) * Dh])

    start_kv(1, 1, 0, NC // 2)
    c_b1.wait()
    wait_all(w1b, wsem.at[4])
    hid = jnp.dot(xn8, w1b[...], preferred_element_type=F32) + b1b[...].astype(F32).reshape(1, -1)
    hid = jax.nn.gelu(hid, approximate=True).astype(BF16)
    c_b2.wait()
    start_kv(1, 1, NC // 2, NC // 2)

    def group(g, carry):
        slot = g % NSLOT
        wait_all(kbuf.at[slot], ksem.at[slot])
        wait_all(vbuf.at[slot], vsem.at[slot])
        for j in range(HG):
            h = (g % NGB) * HG + j
            s = lax.dot_general(qs[h].astype(BF16), kbuf[slot, j], NT,
                                preferred_element_type=F32) * Dh ** -0.5
            p = jnp.exp(s - jnp.max(s, axis=-1, keepdims=True))
            l = jnp.sum(p, axis=-1, keepdims=True)
            o = jnp.dot(p.astype(BF16), vbuf[slot, j], preferred_element_type=F32) / l
            o2 = jnp.concatenate([o, pltpu.roll(o, 6, 0)], axis=1)
            cols = pl.ds(pl.multiple_of(h * 2 * Dh, 2 * Dh), 2 * Dh)
            mine = lax.broadcasted_iota(jnp.int32, o2.shape, 0) == g // NGB
            os_[:, cols] = jnp.where(mine, o2, os_[:, cols])

            @pl.when(g + 2 < NG)
            def _():
                start_kv(g + 2, (g + 2) % NSLOT, j * (NC // HG), NC // HG)

            @pl.when(g + 2 >= NG)
            def _():
                n = Z0 // 32 // (2 * HG)
                start_w(((w2_hbm, w2b, wsem.at[5], 0), (wo_hbm, wob, wsem.at[6], 0)), Z0,
                        ((g + 2 - NG) * HG + j) * n, n)
        return carry

    lax.fori_loop(0, NG, group, 0)

    ob = os_[...].astype(BF16)
    b2 = b2b[...].astype(F32).reshape(1, -1)

    def gate(r0, r1):
        f = lax.dot_general(hid, w2b[r0:r1, :], NT, preferred_element_type=F32) + b2[:, r0:r1]
        return f * jax.nn.sigmoid(f)

    def emit(r0, r1, sem, g):
        wait_all(wob.at[pl.ds(r0, r1 - r0)], sem)
        s = lax.dot_general(ob, wob[r0:r1, :], NT, preferred_element_type=F32)
        o_ref[:, r0:r1] = (x[:, r0:r1] + (s * g)[0:B]).astype(o_ref.dtype)

    cuts = (Z0, Z0 + 128, Z0 + 256, D)
    start_rows(w2_hbm, w2b, wsem.at[7], Z0, D, 0, 3)
    wait_all(w2b.at[pl.ds(0, Z0)], wsem.at[5])
    g0 = gate(0, Z0)
    start_rows(w2_hbm, w2b, wsem.at[7], Z0, D, 3, (D - Z0) // 64 - 3)
    emit(0, Z0, wsem.at[6], g0)
    start_rows(wo_hbm, wob, wsem.at[8], cuts[0], cuts[1])
    start_rows(wo_hbm, wob, wsem.at[9], cuts[1], cuts[2])
    wait_all(w2b.at[pl.ds(Z0, D - Z0)], wsem.at[7])
    g1 = gate(Z0, D)
    start_rows(wo_hbm, wob, wsem.at[10], cuts[2], cuts[3])
    for i in range(3):
        emit(cuts[i], cuts[i + 1], wsem.at[8 + i], g1[:, cuts[i] - Z0:cuts[i + 1] - Z0])


@jax.jit
def pallas_recurrent_scan__sliding_block_cached__dense_activation_gelu__decode_kernel(
    A_x: jax.Array,
    A_k_cache: jax.Array,
    A_v_cache: jax.Array,
    A_wq: jax.Array,
    A_wo: jax.Array,
    B_x: jax.Array,
    B_w1: jax.Array,
    B_b1: jax.Array,
    B_w2: jax.Array,
    B_b2: jax.Array,
):
    B, Sq, D = A_x.shape
    _, Hkv, Sk, Dh = A_k_cache.shape
    W = min(4096, max(256, Sk // 4))
    HD, F = A_wq.shape[1], B_w1.shape[1]
    assert (B, Sq, D) == (2, 1, 576) and HD == 2 * Hkv * Dh and Hkv % HG == 0
    assert W % (R * HG) == 0 and HD % 2048 == 0 and F == 3 * 1536
    dt = A_x.dtype
    out = pl.pallas_call(
        _kernel,
        out_shape=jax.ShapeDtypeStruct((B, D), dt),
        in_specs=[pl.BlockSpec(memory_space=pl.ANY)] * 9,
        out_specs=pl.BlockSpec(memory_space=pltpu.VMEM),
        scratch_shapes=[
            pltpu.VMEM((B, D), dt), pltpu.VMEM((F,), dt), pltpu.VMEM((D,), dt),
            pltpu.VMEM((NSLOT, HG, W, Dh), dt), pltpu.VMEM((NSLOT, HG, W, Dh), dt),
            pltpu.VMEM((D, HD), dt), pltpu.VMEM((D, HD), dt),
            pltpu.VMEM((D, F), dt), pltpu.VMEM((D, F), dt),
            pltpu.VMEM((Hkv, 8, Dh), F32), pltpu.VMEM((8, HD), F32),
            pltpu.SemaphoreType.DMA((NSLOT,)), pltpu.SemaphoreType.DMA((NSLOT,)),
            pltpu.SemaphoreType.DMA((11,)),
        ],
        compiler_params=pltpu.CompilerParams(
            vmem_limit_bytes=64 * 1024 * 1024,
            disable_bounds_checks=True,
            disable_semaphore_checks=True,
        ),
    )(A_x.reshape(B, D), A_k_cache, A_v_cache, A_wq, A_wo.T, B_w1, B_b1, B_w2.T, B_b2)
    return out.reshape(B, Sq, D)
```
